```python
import os as _os
_os.environ.setdefault("JAX_PLATFORMS", "cpu")
import jax
import jax.numpy as jnp

def _softmax(x, axis=-1):
    return jax.nn.softmax(x, axis=axis)
def _gelu(x):
    return jax.nn.gelu(x, approximate=True)
def _silu(x):
    return jax.nn.silu(x)
def _sigmoid(x):
    return jax.nn.sigmoid(x)
def _layernorm(x, axis=-1, eps=1e-5):
    m = jnp.mean(x, axis=axis, keepdims=True)
    v = jnp.var(x, axis=axis, keepdims=True)
    return (x - m) / jnp.sqrt(v + eps)
def _scatter_add(tgt, idx, src, axis=0):
    return tgt.at[idx].add(src)
def _segment_sum(src, seg, n):
    return jax.ops.segment_sum(src, seg, n)
class _Rng:
    def __init__(self, key):
        self._k = key
    def _next(self):
        self._k, sub = jax.random.split(self._k)
        return sub
    def normal(self, shape):
        return jax.random.normal(self._next(), shape, dtype=jnp.bfloat16)
    def randint(self, lo, hi, shape):
        return jax.random.randint(self._next(), shape, lo, hi, dtype=jnp.int32)
    def uniform(self, shape, lo=0.0, hi=1.0):
        return jax.random.uniform(self._next(), shape, jnp.bfloat16, lo, hi)
    def permutation(self, n):
        return jax.random.permutation(self._next(), n)


kernel_name = 'standalone__mha_block_cached__near_ridge'

def setup_inputs():
    _rng = _Rng(jax.random.key(int.from_bytes(__import__("os").urandom(4), "little")))
    _w = (lambda a: (lambda t: t.astype(jnp.bfloat16) if jnp.issubdtype(t.dtype, jnp.floating) else t)(jnp.asarray(a)))
    B, Sq, D = 8, 144, 448
    H, Sk, Dh = 16, 2048, 256
    return {
        "x": _w((lambda *s: _rng.normal(s) * 0.8)(B, Sq, D)),
        "k_cache": _w((lambda *s: _rng.normal(s) * 0.8)(B, H, Sk, Dh)),
        "v_cache": _w((lambda *s: _rng.normal(s) * 0.05)(B, H, Sk, Dh)),
        "wq": _w((lambda *s: _rng.normal(s) * 0.8)(D, H * Dh) * (D ** -0.5)),
        "wo": _w((lambda *s: _rng.normal(s) * 0.05)(H * Dh, D) * ((H * Dh) ** -0.5)),
    }

def reference(x, k_cache, v_cache, wq, wo):
    B, Sq, D = x.shape
    H, Dh = 16, 256
    q = (lambda x, *d: x.transpose(*d))((x @ wq).reshape(B, Sq, H, Dh), 0, 2, 1, 3)
    scores = jnp.einsum("bhqd,bhkd->bhqk", q, k_cache) * (Dh ** -0.5)
    p = _softmax(scores, axis=-1)
    o = jnp.einsum("bhqk,bhkd->bhqd", p, v_cache)
    return (lambda x, *d: x.transpose(*d))(o, 0, 2, 1, 3).reshape(B, Sq, H * Dh) @ wo
```

```python
import functools
import jax
import jax.numpy as jnp
import jax.experimental.pallas as pl
import jax.experimental.pallas.tpu as pltpu

LOG2E = 1.4426950408889634


def _chunks(n, ch):
    out, o = [], 0
    while o < n:
        sz = min(ch, n - o)
        out.append((o, sz))
        o += sz
    return out


def make(NK=4, NV=4, CH=96, LA=55, SKEW=0, SPLIT=11, compute=True, R=1, WCH=112, WLA=3, late_out=True, GRP=100):
  @jax.jit
  def fn(x, k_cache, v_cache, wq, wo):
    B, Sq, D = x.shape
    _, H, Sk, Dh = k_cache.shape
    scale = Dh ** -0.5
    T = B * H
    kf = k_cache.reshape(T, Sk, Dh)
    vf = v_cache.reshape(T, Sk, Dh)
    wot = wo.T
    chunks = _chunks(Sk, CH)
    n = len(chunks)
    wchunks = _chunks(D, WCH)
    assert (LA + n - 1) // n <= NV - 1
    assert (LA + SKEW + n - 1) // n <= NK - 1
    KS, VS = 0, NK
    XS = VS + NV
    QS = XS + B
    WS = QS + H
    OS = WS + H
    NSEM = OS + B

    def kernel(x_hbm, k_hbm, v_hbm, wq_hbm, wot_hbm, o_hbm,
               kbuf, vbuf, xbuf, wqbuf, wobuf, acc, obuf, sem):

        def start_k(t, j):
            o, sz = chunks[j]
            s = t % NK
            pltpu.make_async_copy(k_hbm.at[t % T, pl.ds(o, sz)], kbuf.at[s, pl.ds(o, sz)], sem.at[KS + s]).start(priority=0)

        def start_v(t, j):
            o, sz = chunks[j]
            s = t % NV
            pltpu.make_async_copy(v_hbm.at[t % T, pl.ds(o, sz)], vbuf.at[s, pl.ds(o, sz)], sem.at[VS + s]).start(priority=1)

        def start_w(h):
            off = h * Dh if isinstance(h, int) else pl.multiple_of(h * Dh, Dh)
            for (o, sz) in wchunks:
                pltpu.make_async_copy(wq_hbm.at[pl.ds(o, sz), pl.ds(off, Dh)], wqbuf.at[h, pl.ds(o, sz)], sem.at[QS + h]).start(priority=0)
                pltpu.make_async_copy(wot_hbm.at[pl.ds(o, sz), pl.ds(off, Dh)], wobuf.at[h, pl.ds(o, sz)], sem.at[WS + h]).start(priority=1)

        def x_copy(b):
            return pltpu.make_async_copy(x_hbm.at[b], xbuf.at[b], sem.at[XS + b])

        def out_copy(b):
            return pltpu.make_async_copy(obuf.at[b], o_hbm.at[b], sem.at[OS + b])

        x_copy(0).start(priority=0)
        for c in range(max(LA, LA + SKEW)):
            if c % n == 0 and c // n < WLA:
                start_w(c // n)
            if c < LA + SKEW:
                start_k(c // n, c % n)
            if 0 <= c - max(SKEW, 0) < LA:
                cv = c - max(SKEW, 0)
                start_v(cv // n, cv % n)
        for j in range(-(-max(LA, LA + SKEW) // n), WLA):
            start_w(j)

        def issue(tt, idx):
            groups = []
            for i in idx:
                key = ((LA + SKEW + i) // n, (LA + i) // n)
                if groups and groups[-1][0] == key and len(groups[-1][1]) < GRP:
                    groups[-1][1].append(i)
                else:
                    groups.append((key, [i]))
            for (dk, dv), ii in groups:
                if dk == dv:
                    @pl.when(tt + dk < R * T)
                    def _():
                        for i in ii:
                            start_k(tt + dk, (LA + SKEW + i) % n)
                            start_v(tt + dv, (LA + i) % n)
                else:
                    hi, lo = max(dk, dv), min(dk, dv)
                    @pl.when(tt + hi < R * T)
                    def _():
                        for i in ii:
                            start_k(tt + dk, (LA + SKEW + i) % n)
                            start_v(tt + dv, (LA + i) % n)
                    @pl.when(jnp.logical_and(tt + hi >= R * T, tt + lo < R * T))
                    def _():
                        for i in ii:
                            if dk == lo: start_k(tt + dk, (LA + SKEW + i) % n)
                            else: start_v(tt + dv, (LA + i) % n)

        def body(tt, c):
            t = tt % T
            first = tt < T
            sk = tt % NK
            sv = tt % NV
            b = t // H
            h = t % H

            @pl.when(jnp.logical_and(first, h == 0))
            def _():
                x_copy(b).wait()

            @pl.when(tt < H)
            def _():
                pltpu.make_async_copy(wqbuf.at[h], wqbuf.at[h], sem.at[QS + h]).wait()

            pltpu.make_async_copy(kbuf.at[sk], kbuf.at[sk], sem.at[KS + sk]).wait()

            @pl.when(tt + WLA < H)
            def _():
                start_w(tt + WLA)

            @pl.when(jnp.logical_and(first, jnp.logical_and(h == 8, b + 1 < B)))
            def _():
                x_copy(b + 1).start(priority=0)

            issue(tt, list(range(0, SPLIT)))

            if compute:
                q = jnp.dot(xbuf[b], wqbuf[h], preferred_element_type=jnp.float32)
                q = (q * (scale * LOG2E)).astype(jnp.bfloat16)
                sc = jax.lax.dot_general(q, kbuf[sk], (((1,), (1,)), ((), ())), preferred_element_type=jnp.float32)
                m = jnp.max(sc, axis=-1, keepdims=True)
                p = jnp.exp2(sc - m)
                l = jnp.sum(p, axis=-1, keepdims=True)
                p = p.astype(jnp.bfloat16)

            if late_out:
                @pl.when(tt == R * T - 1)
                def _():
                    for bb in range(B - 1):
                        out_copy(bb).start(priority=1)

            @pl.when(tt < H)
            def _():
                pltpu.make_async_copy(wobuf.at[h], wobuf.at[h], sem.at[WS + h]).wait()
            pltpu.make_async_copy(vbuf.at[sv], vbuf.at[sv], sem.at[VS + sv]).wait()

            issue(tt, list(range(SPLIT, n)))

            if compute:
                o = jnp.dot(p, vbuf[sv], preferred_element_type=jnp.float32)
                o = (o / l).astype(jnp.bfloat16)
                y = jax.lax.dot_general(o, wobuf[h], (((1,), (1,)), ((), ())), preferred_element_type=jnp.float32)
            else:
                y = jnp.zeros((Sq, D), jnp.float32)

            @pl.when(h == 0)
            def _():
                acc[...] = y

            @pl.when(h > 0)
            def _():
                acc[...] += y

            @pl.when(jnp.logical_and(h == H - 1, tt >= (R - 1) * T))
            def _():
                obuf[b] = acc[...].astype(obuf.dtype)
                if late_out:
                    @pl.when(b == B - 1)
                    def _():
                        out_copy(B - 1).start(priority=0)
                else:
                    out_copy(b).start()
            return c

        jax.lax.fori_loop(0, R * T, body, 0)
        for b in range(B):
            out_copy(b).wait()

    hbm = pl.BlockSpec(memory_space=pltpu.HBM)
    return pl.pallas_call(
        kernel,
        in_specs=[hbm] * 5,
        out_specs=hbm,
        out_shape=jax.ShapeDtypeStruct((B, Sq, D), x.dtype),
        scratch_shapes=[
            pltpu.VMEM((NK, Sk, Dh), jnp.bfloat16),
            pltpu.VMEM((NV, Sk, Dh), jnp.bfloat16),
            pltpu.VMEM((B, Sq, D), jnp.bfloat16),
            pltpu.VMEM((H, D, Dh), jnp.bfloat16),
            pltpu.VMEM((H, D, Dh), jnp.bfloat16),
            pltpu.VMEM((Sq, D), jnp.float32),
            pltpu.VMEM((B, Sq, D), jnp.bfloat16),
            pltpu.SemaphoreType.DMA((NSEM,)),
        ],
        compiler_params=pltpu.CompilerParams(
            vmem_limit_bytes=100 * 1024 * 1024,
            disable_bounds_checks=True,
        ),
    )(x, kf, vf, wq, wot)
  return fn

pallas_standalone__mha_block_cached__near_ridge_kernel = make()
```

```python
import functools
import jax
import jax.numpy as jnp
import jax.experimental.pallas as pl
import jax.experimental.pallas.tpu as pltpu

LOG2E = 1.4426950408889634


def _chunks(n, ch):
    out, o = [], 0
    while o < n:
        sz = min(ch, n - o)
        out.append((o, sz))
        o += sz
    return out


def make(S=4, HS=(88, 88, 80), LA=48, SPLIT=12, compute=True, R=1, WR=8, WC=2048, WS=4, XCH=48,
         OCH=144, oprio=1, lastprio=0, pred='item', ST=None, NBUF=None):
  @jax.jit
  def fn(x, k_cache, v_cache, wq, wo):
    B, Sq, D = x.shape
    _, H, Sk, Dh = k_cache.shape
    scale = Dh ** -0.5
    T = B * H
    kf = k_cache.reshape(T, Sk, Dh)
    vf = v_cache.reshape(T, Sk, Dh)
    xf = x.reshape(B * Sq, D)
    wot = wo.T
    streams = ST if ST is not None else tuple((w, S - 1 - w) for w in range(S))
    NP = len(streams)
    W = max(w for w, _ in streams) + 1
    per = Sk // NP
    sizes = []
    while sum(sizes) < per:
        sizes.append(min(HS[len(sizes) % len(HS)], per - sum(sizes)))
    items, o = [], 0
    for z in sizes:
        for (w, p_) in streams:
            items.append((w, p_ * per + o, z))
        o += z
    n = len(items)
    NB = NBUF or ((LA + n - 1) // n + W)
    assert NB >= (LA + n - 1) // n + W
    KS, VS = 0, NB
    XS = VS + NB
    QS = XS + 1
    WSEM = QS + 1
    OS = WSEM + 1
    NSEM = OS + 2

    def kernel(x_hbm, k_hbm, v_hbm, wq_hbm, wot_hbm, o_hbm,
               kbuf, vbuf, xbuf, wqbuf, wobuf, acc, obuf, sem):

        def start_kv(hd, o, sz):
            s = hd % NB
            pltpu.make_async_copy(k_hbm.at[hd % T, pl.ds(o, sz)], kbuf.at[s, pl.ds(o, sz)], sem.at[KS + s]).start(priority=0)
            pltpu.make_async_copy(v_hbm.at[hd % T, pl.ds(o, sz)], vbuf.at[s, pl.ds(o, sz)], sem.at[VS + s]).start(priority=1)

        for i, (o, sz) in enumerate(_chunks(B * Sq, XCH)):
            pltpu.make_async_copy(x_hbm.at[pl.ds(o, sz)], xbuf.at[pl.ds(o, sz)], sem.at[XS]).start(priority=i % 2)
        wper = D // WS
        for (o, sz) in _chunks(wper, WR):
            for (c0, cs) in _chunks(H * Dh, WC):
                for w in range(WS):
                    r = w * wper + o
                    pltpu.make_async_copy(wq_hbm.at[pl.ds(r, sz), pl.ds(c0, cs)], wqbuf.at[pl.ds(r, sz), pl.ds(c0, cs)], sem.at[QS]).start(priority=0)
                    pltpu.make_async_copy(wot_hbm.at[pl.ds(r, sz), pl.ds(c0, cs)], wobuf.at[pl.ds(r, sz), pl.ds(c0, cs)], sem.at[WSEM]).start(priority=1)
        for c in range(-(W - 1) * n, LA):
            g, (w, o, sz) = c // n, items[c % n]
            if g + w >= 0:
                start_kv(g + w, o, sz)
        pltpu.make_async_copy(xbuf, xbuf, sem.at[XS]).wait()
        pltpu.make_async_copy(wqbuf, wqbuf, sem.at[QS]).wait()
        pltpu.make_async_copy(wobuf, wobuf, sem.at[WSEM]).wait()

        def issue(tt, idx):
            if not idx:
                return
            its = []
            for i in idx:
                dg, (w, o, sz) = (LA + i) // n, items[(LA + i) % n]
                its.append((dg + w, o, sz))
            def pred_items():
                for (d, o, sz) in its:
                    @pl.when(tt + d < R * T)
                    def _():
                        start_kv(tt + d, o, sz)
            if pred == 'item':
                pred_items()
            else:
                mx = max(d for d, _, _ in its)
                @pl.when(tt + mx < R * T)
                def _():
                    for (d, o, sz) in its:
                        start_kv(tt + d, o, sz)
                @pl.when(tt + mx >= R * T)
                def _():
                    pred_items()

        NO = (B - 1) * Sq

        def body(tt, c):
            t = tt % T
            sl = tt % NB
            b = t // H
            h = t % H
            row = pl.multiple_of(b * Sq, 16)
            off = pl.multiple_of(h * Dh, Dh)

            pltpu.make_async_copy(kbuf.at[sl], kbuf.at[sl], sem.at[KS + sl]).wait()
            issue(tt, list(range(0, SPLIT)))

            if compute:
                q = jnp.dot(xbuf[pl.ds(row, Sq), :], wqbuf[:, pl.ds(off, Dh)], preferred_element_type=jnp.float32)
                q = (q * (scale * LOG2E)).astype(jnp.bfloat16)
                sc = jax.lax.dot_general(q, kbuf[sl], (((1,), (1,)), ((), ())), preferred_element_type=jnp.float32)
                m = jnp.max(sc, axis=-1, keepdims=True)
                p = jnp.exp2(sc - m)
                l = jnp.sum(p, axis=-1, keepdims=True)
                p = p.astype(jnp.bfloat16)

            @pl.when(tt == R * T - 1)
            def _():
                for i, (o, sz) in enumerate(_chunks(NO, OCH)):
                    pltpu.make_async_copy(obuf.at[pl.ds(o, sz)], o_hbm.at[pl.ds(o, sz)], sem.at[OS]).start(
                        priority=(i % 2 if oprio == 'alt' else oprio))

            pltpu.make_async_copy(vbuf.at[sl], vbuf.at[sl], sem.at[VS + sl]).wait()
            issue(tt, list(range(SPLIT, n)))

            if compute:
                o = jnp.dot(p, vbuf[sl], preferred_element_type=jnp.float32)
                o = (o / l).astype(jnp.bfloat16)
                y = jax.lax.dot_general(o, wobuf[:, pl.ds(off, Dh)], (((1,), (1,)), ((), ())), preferred_element_type=jnp.float32)
            else:
                y = jnp.zeros((Sq, D), jnp.float32)

            @pl.when(h == 0)
            def _():
                acc[...] = y

            @pl.when(h > 0)
            def _():
                acc[...] += y

            @pl.when(h == H - 1)
            def _():
                obuf[pl.ds(row, Sq), :] = acc[...].astype(obuf.dtype)
            return c

        jax.lax.fori_loop(0, R * T, body, 0)
        last = pltpu.make_async_copy(obuf.at[pl.ds(NO, Sq)], o_hbm.at[pl.ds(NO, Sq)], sem.at[OS + 1])
        last.start(priority=lastprio)
        pltpu.make_async_copy(obuf.at[pl.ds(0, NO)], obuf.at[pl.ds(0, NO)], sem.at[OS]).wait()
        last.wait()

    hbm = pl.BlockSpec(memory_space=pltpu.HBM)
    out = pl.pallas_call(
        kernel,
        in_specs=[hbm] * 5,
        out_specs=hbm,
        out_shape=jax.ShapeDtypeStruct((B * Sq, D), x.dtype),
        scratch_shapes=[
            pltpu.VMEM((NB, Sk, Dh), jnp.bfloat16),
            pltpu.VMEM((NB, Sk, Dh), jnp.bfloat16),
            pltpu.VMEM((B * Sq, D), jnp.bfloat16),
            pltpu.VMEM((D, H * Dh), jnp.bfloat16),
            pltpu.VMEM((D, H * Dh), jnp.bfloat16),
            pltpu.VMEM((Sq, D), jnp.float32),
            pltpu.VMEM((B * Sq, D), jnp.bfloat16),
            pltpu.SemaphoreType.DMA((NSEM,)),
        ],
        compiler_params=pltpu.CompilerParams(
            vmem_limit_bytes=100 * 1024 * 1024,
            disable_bounds_checks=True,
        ),
    )(xf, kf, vf, wq, wot)
    return out.reshape(B, Sq, D)
  return fn

pallas_standalone__mha_block_cached__near_ridge_kernel = make(ST=((0, 0), (1, 1), (0, 2), (1, 3)), NBUF=4)
```

```python
import jax
import jax.numpy as jnp
import jax.experimental.pallas as pl
import jax.experimental.pallas.tpu as pltpu

LOG2E = 1.4426950408889634


def _split(lo, n, hs):
    out, o, i = [], 0, 0
    while o < n:
        z = min(hs[i % len(hs)], n - o)
        out.append((lo + o, z))
        o += z
        i += 1
    return out


def _interleave(streams):
    out = []
    for j in range(max(len(s) for s in streams)):
        for s in streams:
            if j < len(s):
                out.append(s[j])
    return out


def _sequence(T, Sk, HS, TU):
    Q = Sk // 4
    seq = []
    for g in range(-1, T):
        st = []
        if g > TU:
            st = [[(g, r, z) for r, z in _split(0, 2 * Q, HS)], [(g, r, z) for r, z in _split(2 * Q, 2 * Q, HS)]]
        else:
            for (w, q) in ((0, 0), (1, 1), (0, 2), (1, 3)):
                if 0 <= g + w <= min(TU, T - 1):
                    st.append([(g + w, r, z) for r, z in _split(q * Q, Q, HS)])
        seq += _interleave(st)
    return seq


def make(HS=(88, 88, 80), LA=44, SPLIT=12, compute=True, WR=8, WC=2048, WS=2, XCH=48,
         OCH=1008, lastprio=0, NB=4, MUK=6, MUV=6, XA=12, L=26, NC=0, LE=26, OPOS=1, oprio=1, pre=False, verbose=False):
  @jax.jit
  def fn(x, k_cache, v_cache, wq, wo):
    B, Sq, D = x.shape
    _, H, Sk, Dh = k_cache.shape
    scale = Dh ** -0.5
    T = B * H
    kf = k_cache.reshape(T, Sk, Dh)
    vf = v_cache.reshape(T, Sk, Dh)
    xf = x.reshape(B * Sq, D)
    wot = wo.T
    NO = (B - 1) * Sq

    xs = [('x', r, z) for r, z in _split(0, B * Sq, (XCH,))]
    wper = D // WS
    ws = [(w * wper + o, z, c, cs) for o, z in _split(0, wper, (WR,)) for c, cs in _split(0, H * Dh, (WC,))
          for w in range(WS)]
    TC = T - NC
    kseq = [('k',) + it for it in _sequence(T, Sk, HS, T - 1 - MUK)]
    vseq = [('v',) + it for it in _sequence(T, Sk, HS, T - 1 - MUV)]
    q0 = xs[:XA] + [('wq',) + it for it in ws] + [it for it in kseq if it[1] < TC]
    q1 = xs[XA:] + [('wo',) + it for it in ws] + [it for it in vseq if it[1] < TC]
    if NC:
        cut = len(q0) - L
        rest = q1[cut:]
        q1 = q1[:cut]
        for hd in range(TC, T):
            rest += [it for it in kseq if it[1] == hd] + [it for it in vseq if it[1] == hd]
        both, alone = rest[:len(rest) - LE], rest[len(rest) - LE:]
        par = len(rest) % 2
        q0 += both[par::2]
        q1 += both[1 - par::2] + alone
    nf = max(len(q0), len(q1))
    fifo = [[(it, p) for it, p in ((q0[f] if f < len(q0) else None, 0), (q1[f] if f < len(q1) else None, 1)) if it]
            for f in range(nf)]
    n = 24
    v0 = len(xs) - XA + len(ws) + n // 2
    c0 = v0 + LA

    def point(t, half):
        lo = c0 + t * n + (SPLIT if half else 0)
        hi = c0 + t * n + (n if half else SPLIT)
        if t == T - 1 and half == 0:
            hi = nf
        if t == T - 1 and half == 1:
            return []
        return [e for pr in fifo[lo:hi] for e in pr]
    main = [point(0, 0), point(0, 1)]
    def shifted(lst, t):
        return [((a, hd + t, r, z), p) for (a, hd, r, z), p in lst]
    assert all(it[0] in 'kv' for hf in (0, 1) for it, _ in main[hf])
    T1 = 0
    while all(point(T1, hf) == shifted(main[hf], T1) for hf in (0, 1)):
        T1 += 1
    for t in range(T):
        for hf in (0, 1):
            for it, _ in point(t, hf):
                if it[0] == 'k':
                    assert it[1] - NB < t or (it[1] - NB == t and hf == 1), (t, hf, it)
                    assert it[1] > t, (t, hf, it)
                elif it[0] == 'v':
                    assert it[1] - NB < t, (t, hf, it)
                    assert it[1] > t or (it[1] == t and (hf == 0 or pre)), (t, hf, it)
                else:
                    assert it[0] == 'o' and t > (B - 1) * H
    prologue = [e for pr in fifo[:c0] for e in pr]
    assert all(it[1] < NB for it, _ in prologue if it[0] in 'kv')
    if verbose:
        print("T1", T1, "len q0", len(q0), "len q1", len(q1), "reads q1", len([i for i in q1 if i[0] != 'o']))

    KS, VS = 0, NB
    XS = VS + NB
    QS = XS + 1
    WSEM = QS + 1
    OS = WSEM + 1
    NSEM = OS + 2

    def kernel(x_hbm, k_hbm, v_hbm, wq_hbm, wot_hbm, o_hbm,
               kbuf, vbuf, xbuf, wqbuf, wobuf, acc, obuf, qbuf, ohbuf, sem):

        def start(it, prio, t=0):
            a = it[0]
            if a in 'kv':
                hd = t + it[1]
                s = hd & (NB - 1)
                src, dst, base = (k_hbm, kbuf, KS) if a == 'k' else (v_hbm, vbuf, VS)
                rows = pl.ds(it[2], it[3])
                cp = pltpu.make_async_copy(src.at[hd, rows], dst.at[s, rows], sem.at[base + s])
            elif a == 'x':
                rows = pl.ds(it[1], it[2])
                cp = pltpu.make_async_copy(x_hbm.at[rows], xbuf.at[rows], sem.at[XS])
            elif a == 'o':
                rows = pl.ds(it[1], it[2])
                cp = pltpu.make_async_copy(obuf.at[rows], o_hbm.at[rows], sem.at[OS])
            else:
                src, dst, si = (wq_hbm, wqbuf, QS) if a == 'wq' else (wot_hbm, wobuf, WSEM)
                rows, cols = pl.ds(it[1], it[2]), pl.ds(it[3], it[4])
                cp = pltpu.make_async_copy(src.at[rows, cols], dst.at[rows, cols], sem.at[si])
            cp.start(priority=prio)

        for it, p in prologue:
            start(it, p)
        acc[...] = jnp.zeros(acc.shape, acc.dtype)
        ohbuf[...] = jnp.zeros(ohbuf.shape, ohbuf.dtype)
        if not compute:
            obuf[...] = jnp.zeros(obuf.shape, obuf.dtype)
        pltpu.make_async_copy(xbuf, xbuf, sem.at[XS]).wait()
        pltpu.make_async_copy(wqbuf, wqbuf, sem.at[QS]).wait()

        def offsets(t):
            if isinstance(t, int):
                return (t // H) * Sq, (t % H) * Dh
            b, h = jax.lax.shift_right_logical(t, 4), t & (H - 1)
            return pl.multiple_of(b * Sq, 16), pl.multiple_of(h * Dh, Dh)

        def qproj(t):
            row, off = offsets(t)
            q = jnp.dot(xbuf[pl.ds(row, Sq), :], wqbuf[:, pl.ds(off, Dh)], preferred_element_type=jnp.float32)
            return (q * (scale * LOG2E)).astype(jnp.bfloat16)

        def outproj(t, keep):
            row, off = offsets(t)
            y = jax.lax.dot_general(ohbuf[...], wobuf[:, pl.ds(off, Dh)], (((1,), (1,)), ((), ())),
                                    preferred_element_type=jnp.float32)
            if keep is True:
                tot = y + acc[...]
            else:
                tot = y + jnp.where(keep, acc[...], 0.0)
                acc[...] = tot
            obuf[pl.ds(row, Sq), :] = tot.astype(obuf.dtype)

        qbuf[...] = qproj(0)
        pltpu.make_async_copy(wobuf, wobuf, sem.at[WSEM]).wait()

        def issue(t, hf):
            def tree(lo, hi):
                if hi - lo == 1:
                    for it, p in point(lo, hf):
                        start(it, p)
                    return
                mid = (lo + hi) // 2
                if any(point(tt, hf) for tt in range(lo, mid)):
                    pl.when(t < mid)(lambda: tree(lo, mid))
                if any(point(tt, hf) for tt in range(mid, hi)):
                    pl.when(t >= mid)(lambda: tree(mid, hi))

            @pl.when(t < T1)
            def _():
                for it, p in main[hf]:
                    start(it, p, t)
            pl.when(t >= T1)(lambda: tree(T1, T))

        def writes(t):
            @pl.when(t == T - 1)
            def _():
                for r, z in _split(0, NO, (OCH,)):
                    start(('o', r, z), oprio)

        def body(t, c):
            sl = t & (NB - 1)
            tp = jnp.maximum(t - 1, 0)
            tn = jnp.minimum(t + 1, T - 1)

            if pre:
                issue(t, 0)
            pltpu.make_async_copy(kbuf.at[sl], kbuf.at[sl], sem.at[KS + sl]).wait()
            if not pre:
                issue(t, 0)
            if OPOS == 0:
                writes(t)

            if compute:
                sc = jax.lax.dot_general(qbuf[...], kbuf[sl], (((1,), (1,)), ((), ())), preferred_element_type=jnp.float32)
                m = jnp.max(sc, axis=-1, keepdims=True)
                qbuf[...] = qproj(tn)
                outproj(tp, (tp & (H - 1)) != 0)

            if OPOS == 1:
                writes(t)
            if pre:
                issue(t, 1)
            pltpu.make_async_copy(vbuf.at[sl], vbuf.at[sl], sem.at[VS + sl]).wait()
            if not pre:
                issue(t, 1)
            if OPOS == 2:
                writes(t)

            if compute:
                p = jnp.exp2(sc - m)
                l = jnp.sum(p, axis=-1, keepdims=True)
                o = jnp.dot(p.astype(jnp.bfloat16), vbuf[sl], preferred_element_type=jnp.float32)
                ohbuf[...] = (o / l).astype(jnp.bfloat16)
            return c

        jax.lax.fori_loop(0, T, body, 0)
        if compute:
            outproj(T - 1, True)
        last = pltpu.make_async_copy(obuf.at[pl.ds(NO, Sq)], o_hbm.at[pl.ds(NO, Sq)], sem.at[OS + 1])
        last.start(priority=lastprio)
        pltpu.make_async_copy(obuf.at[pl.ds(0, NO)], obuf.at[pl.ds(0, NO)], sem.at[OS]).wait()
        last.wait()

    hbm = pl.BlockSpec(memory_space=pltpu.HBM)
    out = pl.pallas_call(
        kernel,
        in_specs=[hbm] * 5,
        out_specs=hbm,
        out_shape=jax.ShapeDtypeStruct((B * Sq, D), x.dtype),
        scratch_shapes=[
            pltpu.VMEM((NB, Sk, Dh), jnp.bfloat16),
            pltpu.VMEM((NB, Sk, Dh), jnp.bfloat16),
            pltpu.VMEM((B * Sq, D), jnp.bfloat16),
            pltpu.VMEM((D, H * Dh), jnp.bfloat16),
            pltpu.VMEM((D, H * Dh), jnp.bfloat16),
            pltpu.VMEM((Sq, D), jnp.float32),
            pltpu.VMEM((B * Sq, D), jnp.bfloat16),
            pltpu.VMEM((Sq, Dh), jnp.bfloat16),
            pltpu.VMEM((Sq, Dh), jnp.bfloat16),
            pltpu.SemaphoreType.DMA((NSEM,)),
        ],
        compiler_params=pltpu.CompilerParams(
            vmem_limit_bytes=100 * 1024 * 1024,
            disable_bounds_checks=True,
        ),
    )(xf, kf, vf, wq, wot)
    return out.reshape(B, Sq, D)
  return fn

pallas_standalone__mha_block_cached__near_ridge_kernel = make(NC=2, NB=8, XA=18, MUK=5, MUV=5)
```

```python
import jax
import jax.numpy as jnp
import jax.experimental.pallas as pl
import jax.experimental.pallas.tpu as pltpu

LOG2E = 1.4426950408889634


def _split(lo, n, hs):
    out, o, i = [], 0, 0
    while o < n:
        z = min(hs[i % len(hs)], n - o)
        out.append((lo + o, z))
        o += z
        i += 1
    return out


def _interleave(streams):
    out = []
    for j in range(max(len(s) for s in streams)):
        for s in streams:
            if j < len(s):
                out.append(s[j])
    return out


def _head_parts(Sk, PH, SM, NP, mode):
    bnd = sorted(set([0, Sk] + [r for r in range(1, Sk) if (r - PH) % 128 in (0, SM)]))
    parts = [[] for _ in range(NP)]
    for a, b in zip(bnd[:-1], bnd[1:]):
        small = (a - PH) % 128 == 0
        if small and mode == 'strided':
            continue
        parts[min(NP - 1, max(0, ((a + b) // 2 - PH) * NP // Sk))].append((a, b - a))
    return parts


def _sequence(T, Sk, PH, SM, TU, mode, SPOS):
    P4 = _head_parts(Sk, PH, SM, 4, mode)
    P2 = _head_parts(Sk, PH, SM, 2, mode)
    seq, starts = [], {}
    for g in range(-1, T):
        starts[g] = len(seq)
        st = []
        if g > TU:
            st = [[(g, r, z) for r, z in p] for p in P2]
        else:
            for (w, q) in ((0, 0), (1, 1), (0, 2), (1, 3)):
                if 0 <= g + w <= min(TU, T - 1):
                    st.append([(g + w, r, z) for r, z in P4[q]])
        gen = _interleave(st)
        if mode == 'strided' and g >= 0:
            gen.insert(SPOS, (g, -1, 0))
        seq += gen
    return seq, starts


def make(PH=48, SM=8, mode='rr', SPOS=1, LA=60, SPLIT=16, compute=True, WR=8, WC=(1664, 2432), WS=4, XCH=48,
         OCH=1008, lastprio=0, NB=8, MUK=5, MUV=5, XA=17, L=26, NC=2, LE=26, OPOS=1, oprio=1, pre=False, verbose=False):
  @jax.jit
  def fn(x, k_cache, v_cache, wq, wo):
    B, Sq, D = x.shape
    _, H, Sk, Dh = k_cache.shape
    scale = Dh ** -0.5
    T = B * H
    kf = k_cache.reshape(T, Sk, Dh)
    vf = v_cache.reshape(T, Sk, Dh)
    xf = x.reshape(B * Sq, D)
    wot = wo.T
    NO = (B - 1) * Sq

    xs = [('x', r, z) for r, z in _split(0, B * Sq, (XCH,))]
    wper = D // WS
    ws = [(w * wper + o, z, c, cs) for o, z in _split(0, wper, (WR,)) for c, cs in _split(0, H * Dh, WC)
          for w in range(WS)]
    TC = T - NC
    kseq, starts = _sequence(T, Sk, PH, SM, T - 1 - MUK, mode, SPOS)
    vseq, starts = _sequence(T, Sk, PH, SM, T - 1 - MUV, mode, SPOS)
    kseq = [('k',) + it for it in kseq]
    vseq = [('v',) + it for it in vseq]
    q0 = xs[:XA] + [('wq',) + it for it in ws] + [it for it in kseq if it[1] < TC]
    q1 = xs[XA:] + [('wo',) + it for it in ws] + [it for it in vseq if it[1] < TC]
    if NC:
        cut = len(q0) - L
        rest = q1[cut:]
        q1 = q1[:cut]
        for hd in range(TC, T):
            rest += [it for it in kseq if it[1] == hd] + [it for it in vseq if it[1] == hd]
        both, alone = rest[:len(rest) - LE], rest[len(rest) - LE:]
        par = len(rest) % 2
        q0 += both[par::2]
        q1 += both[1 - par::2] + alone
    nf = max(len(q0), len(q1))
    fifo = [[(it, p) for it, p in ((q0[f] if f < len(q0) else None, 0), (q1[f] if f < len(q1) else None, 1)) if it]
            for f in range(nf)]
    n = starts[1] - starts[0]
    v0 = len(xs) - XA + len(ws) + starts[0]
    c0 = v0 + LA

    def point(t, half):
        lo = c0 + t * n + (SPLIT if half else 0)
        hi = c0 + t * n + (n if half else SPLIT)
        if t == T - 1 and half == 0:
            hi = nf
        if t == T - 1 and half == 1:
            return []
        return [e for pr in fifo[lo:hi] for e in pr]
    main = [point(0, 0), point(0, 1)]
    def shifted(lst, t):
        return [((a, hd + t, r, z), p) for (a, hd, r, z), p in lst]
    assert all(it[0] in 'kv' for hf in (0, 1) for it, _ in main[hf])
    T1 = 0
    while all(point(T1, hf) == shifted(main[hf], T1) for hf in (0, 1)):
        T1 += 1
    for t in range(T):
        for hf in (0, 1):
            for it, _ in point(t, hf):
                if it[0] == 'k':
                    assert it[1] - NB < t or (it[1] - NB == t and hf == 1), (t, hf, it)
                    assert it[1] > t, (t, hf, it)
                elif it[0] == 'v':
                    assert it[1] - NB < t, (t, hf, it)
                    assert it[1] > t or (it[1] == t and (hf == 0 or pre)), (t, hf, it)
                else:
                    assert it[0] == 'o' and t > (B - 1) * H
    prologue = [e for pr in fifo[:c0] for e in pr]
    assert all(it[1] < NB for it, _ in prologue if it[0] in 'kv')
    if verbose:
        print("n", n, "T1", T1, "len q0", len(q0), "len q1", len(q1), "reads q1", len([i for i in q1 if i[0] != 'o']))

    KS, VS = 0, NB
    XS = VS + NB
    QS = XS + 1
    WSEM = QS + 1
    OS = WSEM + 1
    NSEM = OS + 2

    def kernel(x_hbm, k_hbm, v_hbm, wq_hbm, wot_hbm, o_hbm,
               kbuf, vbuf, xbuf, wqbuf, wobuf, acc, obuf, qbuf, ohbuf, sem):

        def start(it, prio, t=0):
            a = it[0]
            if a in 'kv':
                hd = t + it[1]
                s = hd & (NB - 1)
                src, dst, base = (k_hbm, kbuf, KS) if a == 'k' else (v_hbm, vbuf, VS)
                if it[2] >= 0:
                    rows = pl.ds(it[2], it[3])
                    cp = pltpu.make_async_copy(src.at[hd, rows], dst.at[s, rows], sem.at[base + s])
                else:
                    rows = pl.ds(PH, SM)
                    cp = pltpu.make_async_copy(src.at[hd].reshape(Sk // 128, 128, Dh).at[:, rows],
                                               dst.at[s].reshape(Sk // 128, 128, Dh).at[:, rows], sem.at[base + s])
            elif a == 'x':
                rows = pl.ds(it[1], it[2])
                cp = pltpu.make_async_copy(x_hbm.at[rows], xbuf.at[rows], sem.at[XS])
            elif a == 'o':
                rows = pl.ds(it[1], it[2])
                cp = pltpu.make_async_copy(obuf.at[rows], o_hbm.at[rows], sem.at[OS])
            else:
                src, dst, si = (wq_hbm, wqbuf, QS) if a == 'wq' else (wot_hbm, wobuf, WSEM)
                rows, cols = pl.ds(it[1], it[2]), pl.ds(it[3], it[4])
                cp = pltpu.make_async_copy(src.at[rows, cols], dst.at[rows, cols], sem.at[si])
            cp.start(priority=prio)

        for it, p in prologue:
            start(it, p)
        acc[...] = jnp.zeros(acc.shape, acc.dtype)
        ohbuf[...] = jnp.zeros(ohbuf.shape, ohbuf.dtype)
        if not compute:
            obuf[...] = jnp.zeros(obuf.shape, obuf.dtype)
        pltpu.make_async_copy(xbuf, xbuf, sem.at[XS]).wait()
        pltpu.make_async_copy(wqbuf, wqbuf, sem.at[QS]).wait()

        def offsets(t):
            if isinstance(t, int):
                return (t // H) * Sq, (t % H) * Dh
            b, h = jax.lax.shift_right_logical(t, 4), t & (H - 1)
            return pl.multiple_of(b * Sq, 16), pl.multiple_of(h * Dh, Dh)

        def qproj(t):
            row, off = offsets(t)
            q = jnp.dot(xbuf[pl.ds(row, Sq), :], wqbuf[:, pl.ds(off, Dh)], preferred_element_type=jnp.float32)
            return (q * (scale * LOG2E)).astype(jnp.bfloat16)

        def outproj(t, keep):
            row, off = offsets(t)
            y = jax.lax.dot_general(ohbuf[...], wobuf[:, pl.ds(off, Dh)], (((1,), (1,)), ((), ())),
                                    preferred_element_type=jnp.float32)
            if keep is True:
                tot = y + acc[...]
            else:
                tot = y + jnp.where(keep, acc[...], 0.0)
                acc[...] = tot
            obuf[pl.ds(row, Sq), :] = tot.astype(obuf.dtype)

        qbuf[...] = qproj(0)
        pltpu.make_async_copy(wobuf, wobuf, sem.at[WSEM]).wait()

        def issue(t, hf):
            def tree(lo, hi):
                if hi - lo == 1:
                    for it, p in point(lo, hf):
                        start(it, p)
                    return
                mid = (lo + hi) // 2
                if any(point(tt, hf) for tt in range(lo, mid)):
                    pl.when(t < mid)(lambda: tree(lo, mid))
                if any(point(tt, hf) for tt in range(mid, hi)):
                    pl.when(t >= mid)(lambda: tree(mid, hi))

            @pl.when(t < T1)
            def _():
                for it, p in main[hf]:
                    start(it, p, t)
            pl.when(t >= T1)(lambda: tree(T1, T))

        def writes(t):
            @pl.when(t == T - 1)
            def _():
                for r, z in _split(0, NO, (OCH,)):
                    start(('o', r, z), oprio)

        def body(t, c):
            sl = t & (NB - 1)
            tp = jnp.maximum(t - 1, 0)
            tn = jnp.minimum(t + 1, T - 1)

            if pre:
                issue(t, 0)
            pltpu.make_async_copy(kbuf.at[sl], kbuf.at[sl], sem.at[KS + sl]).wait()
            if not pre:
                issue(t, 0)
            if OPOS == 0:
                writes(t)

            if compute:
                sc = jax.lax.dot_general(qbuf[...], kbuf[sl], (((1,), (1,)), ((), ())), preferred_element_type=jnp.float32)
                m = jnp.max(sc, axis=-1, keepdims=True)
                qbuf[...] = qproj(tn)
                outproj(tp, (tp & (H - 1)) != 0)

            if OPOS == 1:
                writes(t)
            if pre:
                issue(t, 1)
            pltpu.make_async_copy(vbuf.at[sl], vbuf.at[sl], sem.at[VS + sl]).wait()
            if not pre:
                issue(t, 1)
            if OPOS == 2:
                writes(t)

            if compute:
                p = jnp.exp2(sc - m)
                l = jnp.sum(p, axis=-1, keepdims=True)
                o = jnp.dot(p.astype(jnp.bfloat16), vbuf[sl], preferred_element_type=jnp.float32)
                ohbuf[...] = (o / l).astype(jnp.bfloat16)
            return c

        jax.lax.fori_loop(0, T, body, 0)
        if compute:
            outproj(T - 1, True)
        last = pltpu.make_async_copy(obuf.at[pl.ds(NO, Sq)], o_hbm.at[pl.ds(NO, Sq)], sem.at[OS + 1])
        last.start(priority=lastprio)
        pltpu.make_async_copy(obuf.at[pl.ds(0, NO)], obuf.at[pl.ds(0, NO)], sem.at[OS]).wait()
        last.wait()

    hbm = pl.BlockSpec(memory_space=pltpu.HBM)
    out = pl.pallas_call(
        kernel,
        in_specs=[hbm] * 5,
        out_specs=hbm,
        out_shape=jax.ShapeDtypeStruct((B * Sq, D), x.dtype),
        scratch_shapes=[
            pltpu.VMEM((NB, Sk, Dh), jnp.bfloat16),
            pltpu.VMEM((NB, Sk, Dh), jnp.bfloat16),
            pltpu.VMEM((B * Sq, D), jnp.bfloat16),
            pltpu.VMEM((D, H * Dh), jnp.bfloat16),
            pltpu.VMEM((D, H * Dh), jnp.bfloat16),
            pltpu.VMEM((Sq, D), jnp.float32),
            pltpu.VMEM((B * Sq, D), jnp.bfloat16),
            pltpu.VMEM((Sq, Dh), jnp.bfloat16),
            pltpu.VMEM((Sq, Dh), jnp.bfloat16),
            pltpu.SemaphoreType.DMA((NSEM,)),
        ],
        compiler_params=pltpu.CompilerParams(
            vmem_limit_bytes=100 * 1024 * 1024,
            disable_bounds_checks=True,
        ),
    )(xf, kf, vf, wq, wot)
    return out.reshape(B, Sq, D)
  return fn

pallas_standalone__mha_block_cached__near_ridge_kernel = make(mode='strided', LA=44, SPLIT=9, XA=19, SPOS=8, MUK=6, MUV=6)
```

```python
import jax
import jax.numpy as jnp
import jax.experimental.pallas as pl
import jax.experimental.pallas.tpu as pltpu

LOG2E = 1.4426950408889634


def _split(lo, n, hs):
    out, o, i = [], 0, 0
    while o < n:
        z = min(hs[i % len(hs)], n - o)
        out.append((lo + o, z))
        o += z
        i += 1
    return out


def _interleave(streams):
    out = []
    for j in range(max(len(s) for s in streams)):
        for s in streams:
            if j < len(s):
                out.append(s[j])
    return out


def _sequence(T, NT, PT, TU, QO, HO, whole):
    def visit(hd, s):
        lo = PT + 32 * (s - 1)
        if whole(s):
            return [(hd, lo, 32)]
        a, b = (hd, lo, 32 - PT), (hd, lo + 32 - PT, PT)
        if s == NT // 32:
            b = (hd + 1, 0, PT)
        return [p for p in (a, b) if 0 <= p[0] < T]
    seq, starts = visit(-1, NT // 32), {}
    for g in range(-1, T):
        starts[g] = len(seq)
        if g > TU:
            st = [[visit(g, s) for s in q] for q in HO]
        else:
            st = [[visit(g + w, s) for s in q] for w, q in zip((0, 1, 0, 1), QO) if 0 <= g + w <= min(TU, T - 1)]
        seq += [p for v in _interleave(st) for p in v]
    return seq, starts


def make(PT=13, LA=44, SPLIT=12, compute=True, WS=4, XCH=48, VR=64, WH='odd',
         QO=((1, 2, 3, 4), (6, 5, 8, 7), (9, 10, 11, 12), (14, 13, 16, 15)),
         HO=((1, 2, 3, 4, 5, 6, 7, 8), (10, 9, 12, 11, 14, 13, 16, 15)),
         OCH=1008, lastprio=0, NB=8, MUK=6, MUV=6, XA=7, L=26, NC=2, LE=26, OPOS=1, oprio=1, pre=False,
         verbose=False, NOSEM=True, PAD=26, RED=0, RS=7, RMAX=0):
  @jax.jit
  def fn(x, k_cache, v_cache, wq, wo):
    B, Sq, D = x.shape
    _, H, Sk, Dh = k_cache.shape
    scale = Dh ** -0.5
    T = B * H
    NG = Sk // VR
    TPR = NG * Dh // 128
    wide = lambda a: a.reshape(T, VR // 8, NG, 8, Dh).transpose(0, 1, 3, 2, 4).reshape(T, VR, NG * Dh)
    kf, vf = wide(k_cache), wide(v_cache)
    xf = x.reshape(B * Sq, D)
    wot = wo.T
    NO = (B - 1) * Sq
    NT = Sk * Dh // 1024

    whole = {'odd': lambda s: s % 2 == 1, 'none': lambda s: False, 'all': lambda s: s % 8 != 0,
             'q3': lambda s: s % 4 == 1}[WH]
    xs = [('x', r, z) for r, z in _split(0, B * Sq, (XCH,))]
    CUT, WR = PT * 128, D // 8
    def wstripe(i):
        return ([(8 * i, CUT, H * Dh - CUT)] if i >= 0 else []) + ([(8 * i + 8, 0, CUT)] if i + 1 < WR else [])
    wper = WR // WS
    ws = wstripe(-1) + [p for v in _interleave([[wstripe(w * wper + i) for i in range(wper)] for w in range(WS)])
                        for p in v]
    TC = T - NC
    kseq, starts = _sequence(T, NT, PT, T - 1 - MUK, QO, HO, whole)
    vseq, starts = _sequence(T, NT, PT, T - 1 - MUV, QO, HO, whole)
    kseq = [('k',) + it for it in kseq]
    vseq = [('v',) + it for it in vseq]
    q0 = [None] * PAD + xs[:XA] + [('wq',) + it for it in ws] + [it for it in kseq if it[1] < TC]
    q1 = xs[XA:] + [('wo',) + it for it in ws] + [it for it in vseq if it[1] < TC]
    if NC:
        cut = len(q0) - L
        rest = q1[cut:]
        q1 = q1[:cut]
        for hd in range(TC, T):
            rest += [it for it in kseq if it[1] == hd] + [it for it in vseq if it[1] == hd]
        both, alone = rest[:len(rest) - LE], rest[len(rest) - LE:]
        q0 += [it for it in both if it[2] < NT // 2]
        q1 += [it for it in both if it[2] >= NT // 2] + alone
    nf = max(len(q0), len(q1))
    fifo = [[(it, p) for it, p in ((q0[f] if f < len(q0) else None, 0), (q1[f] if f < len(q1) else None, 1)) if it]
            for f in range(nf)]
    n = starts[1] - starts[0]
    v0 = len(xs) - XA + len(ws) + starts[0]
    c0 = v0 + LA

    def pos(p):
        t, half = p // 2, p % 2
        if p >= 2 * T - 1:
            return nf
        red = min(RMAX, max(0, p - 2 * (T - RS)) * RED)
        return min(nf, c0 + t * n + (SPLIT if half else 0) - red)

    def point(t, half):
        return [e for pr in fifo[pos(2 * t + half):pos(2 * t + half + 1)] for e in pr]
    main = [point(0, 0), point(0, 1)]
    def shifted(lst, t):
        return [((a, hd + t, r, z), p) for (a, hd, r, z), p in lst]
    assert all(it[0] in 'kv' for hf in (0, 1) for it, _ in main[hf])
    T1 = 0
    while all(point(T1, hf) == shifted(main[hf], T1) for hf in (0, 1)):
        T1 += 1
    for t in range(T):
        for hf in (0, 1):
            for it, _ in point(t, hf):
                assert it[0] in 'kv' and it[1] - NB < t, (t, hf, it)
                assert it[1] > t or (it[0] == 'v' and it[1] == t and (hf == 0 or pre)), (t, hf, it)
    prologue = [e for pr in fifo[:c0] for e in pr]
    assert all(it[1] < NB for it, _ in prologue if it[0] in 'kv')
    for a in 'kv':
        got = sorted((it[1], it[2], it[3]) for pr in fifo for it, _ in pr if it[0] == a)
        at = 0
        for hd, o, z in got:
            assert hd * NT + o == at and o // TPR == (o + z - 1) // TPR
            at += z
        assert at == T * NT
    if verbose:
        print("n", n, "T1", T1, "len q0", len(q0), "len q1", len(q1))

    KS, VS = 0, NB
    XS = VS + NB
    QS = XS + 1
    WSEM = QS + 1
    OS = WSEM + 1
    NSEM = OS + 2

    def kernel(x_hbm, k_hbm, v_hbm, wq_hbm, wot_hbm, o_hbm,
               kbuf, vbuf, xbuf, wqbuf, wobuf, acc, obuf, qbuf, ohbuf, sem):

        def start(it, prio, t=0):
            a = it[0]
            if a in 'kv':
                hd = t + it[1]
                s = hd & (NB - 1)
                src, dst, base = (k_hbm, kbuf, KS) if a == 'k' else (v_hbm, vbuf, VS)
                rows, cols = pl.ds(8 * (it[2] // TPR), 8), pl.ds(128 * (it[2] % TPR), 128 * it[3])
                cp = pltpu.make_async_copy(src.at[hd, rows, cols], dst.at[s, rows, cols], sem.at[base + s])
            elif a == 'x':
                rows = pl.ds(it[1], it[2])
                cp = pltpu.make_async_copy(x_hbm.at[rows], xbuf.at[rows], sem.at[XS])
            elif a == 'o':
                rows = pl.ds(it[1], it[2])
                cp = pltpu.make_async_copy(obuf.at[rows], o_hbm.at[rows], sem.at[OS])
            else:
                src, dst, si = (wq_hbm, wqbuf, QS) if a == 'wq' else (wot_hbm, wobuf, WSEM)
                rows, cols = pl.ds(it[1], 8), pl.ds(it[2], it[3])
                cp = pltpu.make_async_copy(src.at[rows, cols], dst.at[rows, cols], sem.at[si])
            cp.start(priority=prio)

        for it, p in prologue:
            start(it, p)
        acc[...] = jnp.zeros(acc.shape, acc.dtype)
        ohbuf[...] = jnp.zeros(ohbuf.shape, ohbuf.dtype)
        if not compute:
            obuf[...] = jnp.zeros(obuf.shape, obuf.dtype)
        pltpu.make_async_copy(xbuf, xbuf, sem.at[XS]).wait()
        pltpu.make_async_copy(wqbuf, wqbuf, sem.at[QS]).wait()

        def offsets(t):
            if isinstance(t, int):
                return (t // H) * Sq, (t % H) * Dh
            b, h = jax.lax.shift_right_logical(t, 4), t & (H - 1)
            return pl.multiple_of(b * Sq, 16), pl.multiple_of(h * Dh, Dh)

        def keys(buf, sl):
            return jnp.concatenate([buf[sl, :, g * Dh:(g + 1) * Dh] for g in range(NG)], axis=0)

        def qproj(t):
            row, off = offsets(t)
            q = jnp.dot(xbuf[pl.ds(row, Sq), :], wqbuf[:, pl.ds(off, Dh)], preferred_element_type=jnp.float32)
            return (q * (scale * LOG2E)).astype(jnp.bfloat16)

        def outproj(t, keep):
            row, off = offsets(t)
            y = jax.lax.dot_general(ohbuf[...], wobuf[:, pl.ds(off, Dh)], (((1,), (1,)), ((), ())),
                                    preferred_element_type=jnp.float32)
            if keep is True:
                tot = y + acc[...]
            else:
                tot = y + jnp.where(keep, acc[...], 0.0)
                acc[...] = tot
            obuf[pl.ds(row, Sq), :] = tot.astype(obuf.dtype)

        qbuf[...] = qproj(0)
        pltpu.make_async_copy(wobuf, wobuf, sem.at[WSEM]).wait()

        def issue(t, hf):
            def tree(lo, hi):
                if hi - lo == 1:
                    for it, p in point(lo, hf):
                        start(it, p)
                    return
                mid = (lo + hi) // 2
                if any(point(tt, hf) for tt in range(lo, mid)):
                    pl.when(t < mid)(lambda: tree(lo, mid))
                if any(point(tt, hf) for tt in range(mid, hi)):
                    pl.when(t >= mid)(lambda: tree(mid, hi))

            @pl.when(t < T1)
            def _():
                for it, p in main[hf]:
                    start(it, p, t)
            pl.when(t >= T1)(lambda: tree(T1, T))

        def writes(t):
            @pl.when(t == T - 1)
            def _():
                for r, z in _split(0, NO, (OCH,)):
                    start(('o', r, z), oprio)

        def body(t, c):
            sl = t & (NB - 1)
            tp = jnp.maximum(t - 1, 0)
            tn = jnp.minimum(t + 1, T - 1)

            if pre:
                issue(t, 0)
            pltpu.make_async_copy(kbuf.at[sl], kbuf.at[sl], sem.at[KS + sl]).wait()
            if not pre:
                issue(t, 0)
            if OPOS == 0:
                writes(t)

            if compute:
                sc = jax.lax.dot_general(qbuf[...], keys(kbuf, sl), (((1,), (1,)), ((), ())),
                                         preferred_element_type=jnp.float32)
                m = jnp.max(sc, axis=-1, keepdims=True)
                qbuf[...] = qproj(tn)
                outproj(tp, (tp & (H - 1)) != 0)

            if OPOS == 1:
                writes(t)
            if pre:
                issue(t, 1)
            pltpu.make_async_copy(vbuf.at[sl], vbuf.at[sl], sem.at[VS + sl]).wait()
            if not pre:
                issue(t, 1)
            if OPOS == 2:
                writes(t)

            if compute:
                p = jnp.exp2(sc - m)
                l = jnp.sum(p, axis=-1, keepdims=True)
                o = jnp.dot(p.astype(jnp.bfloat16), keys(vbuf, sl), preferred_element_type=jnp.float32)
                ohbuf[...] = (o / l).astype(jnp.bfloat16)
            return c

        jax.lax.fori_loop(0, T, body, 0)
        if compute:
            outproj(T - 1, True)
        last = pltpu.make_async_copy(obuf.at[pl.ds(NO, Sq)], o_hbm.at[pl.ds(NO, Sq)], sem.at[OS + 1])
        last.start(priority=lastprio)
        pltpu.make_async_copy(obuf.at[pl.ds(0, NO)], obuf.at[pl.ds(0, NO)], sem.at[OS]).wait()
        last.wait()

    hbm = pl.BlockSpec(memory_space=pltpu.HBM)
    out = pl.pallas_call(
        kernel,
        in_specs=[hbm] * 5,
        out_specs=hbm,
        out_shape=jax.ShapeDtypeStruct((B * Sq, D), x.dtype),
        scratch_shapes=[
            pltpu.VMEM((NB, VR, NG * Dh), jnp.bfloat16),
            pltpu.VMEM((NB, VR, NG * Dh), jnp.bfloat16),
            pltpu.VMEM((B * Sq, D), jnp.bfloat16),
            pltpu.VMEM((D, H * Dh), jnp.bfloat16),
            pltpu.VMEM((D, H * Dh), jnp.bfloat16),
            pltpu.VMEM((Sq, D), jnp.float32),
            pltpu.VMEM((B * Sq, D), jnp.bfloat16),
            pltpu.VMEM((Sq, Dh), jnp.bfloat16),
            pltpu.VMEM((Sq, Dh), jnp.bfloat16),
            pltpu.SemaphoreType.DMA((NSEM,)),
        ],
        compiler_params=pltpu.CompilerParams(
            vmem_limit_bytes=100 * 1024 * 1024,
            disable_bounds_checks=True,
            disable_semaphore_checks=NOSEM,
        ),
    )(xf, kf, vf, wq, wot)
    return out.reshape(B, Sq, D)
  return fn

pallas_standalone__mha_block_cached__near_ridge_kernel = make(WH='none', VR=128, SPLIT=16, XA=4, RS=7, LA=54, RED=3, RMAX=16)
```

```python
import jax
import jax.numpy as jnp
import jax.experimental.pallas as pl
import jax.experimental.pallas.tpu as pltpu


_STRIPE = 32
_PHASE = 13
_NBUF = 8
_LEAD = 26
_AHEAD = 56
_X_ROWS = 48
_X_Q0 = 4
_W_STREAMS = 4
_DEPTHS = ((7, 1), (18, 2), (1 << 30, 4))
_N_SERIAL = 2
_COST_A, _COST_B = 16, 13


def _interleave(streams):
    return [s[j] for j in range(max(len(s) for s in streams)) for s in streams if j < len(s)]


def _kv_order(n_heads, n_stripes):
    def visit(hd, s):
        nxt = (hd, s + 1) if s + 1 < n_stripes else (hd + 1, 0)
        both = [(hd, s, _PHASE, _STRIPE - _PHASE), nxt + (0, _PHASE)]
        return [p for p in both if 0 <= p[0] < n_heads]

    def depth(hd):
        return next(d for n, d in _DEPTHS if n_heads - hd <= n)

    half = n_stripes // 2
    order, starts = visit(-1, n_stripes - 1), {}
    deepest = _DEPTHS[-1][1]
    for g in range(1 - deepest, n_heads):
        starts[g] = len(order)
        work = []
        for i in range(2):
            for w in range(deepest):
                hd = g + w
                if 0 <= hd < n_heads and w < depth(hd):
                    lo, hi = w * half // depth(hd), (w + 1) * half // depth(hd)
                    for j in range(lo, hi):
                        work.append(((j - lo + 0.5) / (hi - lo), len(work), visit(hd, i * half + j)))
        order += [p for _, _, v in sorted(work) for p in v]
    return order, starts


def _schedule(n_heads, n_stripes, x_rows, w_rows, w_tiles):
    assert w_tiles == _STRIPE
    xs = [('x', r, min(_X_ROWS, x_rows - r)) for r in range(0, x_rows, _X_ROWS)]

    def w_visit(i):
        both = [(i, _PHASE, _STRIPE - _PHASE), (i + 1, 0, _PHASE)]
        return [p for p in both if 0 <= p[0] < w_rows]

    band = w_rows // _W_STREAMS
    ws = w_visit(-1) + [p for v in _interleave(
        [[w_visit(i * band + j) for j in range(band)] for i in range(_W_STREAMS)]) for p in v]
    order, starts = _kv_order(n_heads, n_stripes)
    serial = n_heads - _N_SERIAL
    q0 = [None] * _LEAD + xs[:_X_Q0] + [('wq',) + p for p in ws] + [('k',) + p for p in order if p[0] < serial]
    q1 = xs[_X_Q0:] + [('wo',) + p for p in ws] + [('v',) + p for p in order if p[0] < serial]
    cut = len(q0) - _LEAD
    rest, q1 = q1[cut:], q1[:cut]
    for hd in range(serial, n_heads):
        rest += [(a,) + p for a in 'kv' for p in order if p[0] == hd]
    shared, alone = rest[:-_LEAD], rest[-_LEAD:]
    q0 += [c for c in shared if c[2] < n_stripes // 2]
    q1 += [c for c in shared if c[2] >= n_stripes // 2] + alone
    n_slots = max(len(q0), len(q1))
    slots = [[(q[f], i) for i, q in enumerate((q0, q1)) if f < len(q) and q[f]] for f in range(n_slots)]

    ready = {}
    for f, s in enumerate(slots):
        for c, queue in s:
            ready[c[:2]] = max(ready.get(c[:2], 0), f + 1 - (_LEAD if queue == 0 else 0))
    upto, now = [], 0
    for t in range(n_heads):
        now = max(now, ready['k', t])
        upto.append(now + _AHEAD)
        now = max(now + _COST_A, ready['v', t])
        upto.append(now + _AHEAD)
        now += _COST_B
    per_step = starts[1] - starts[0]
    upto[0] = upto[2] - per_step
    first = upto[1] - per_step
    upto = [first] + [min(u, n_slots) for u in upto[:-2]] + [n_slots, n_slots]

    def point(t, half):
        return [c for s in slots[upto[2 * t + half]:upto[2 * t + half + 1]] for c in s]

    prologue = [c for s in slots[:first] for c in s]
    assert upto == sorted(upto) and band * _W_STREAMS == w_rows
    assert all(c[1] < _NBUF for c, _ in prologue if c[0] in 'kv')
    for t in range(n_heads):
        for half in (0, 1):
            for c, _ in point(t, half):
                assert c[0] in 'kv' and c[1] - _NBUF < t
                assert c[1] > t or (c[0] == 'v' and c[1] == t and half == 0)
    for a in 'kv':
        at = 0
        for hd, row, lo, n in sorted(c[1:] for s in slots for c, _ in s if c[0] == a):
            assert (hd * n_stripes + row) * _STRIPE + lo == at
            at += n
        assert at == n_heads * n_stripes * _STRIPE
    return prologue, point


@jax.jit
def pallas_standalone__mha_block_cached__near_ridge_kernel(
    x: jax.Array,
    k_cache: jax.Array,
    v_cache: jax.Array,
    wq: jax.Array,
    wo: jax.Array,
):
    B, Sq, D = x.shape
    _, H, Sk, Dh = k_cache.shape
    T = B * H
    assert H & (H - 1) == 0 and Sq % 16 == 0 and D % 8 == 0
    n_groups = _STRIPE * 128 // Dh
    n_stripes = Sk // (8 * n_groups)
    q_scale = Dh ** -0.5
    n_early = (B - 1) * Sq

    def wide(a):
        a = a.reshape(T, n_stripes, n_groups, 8, Dh).transpose(0, 1, 3, 2, 4)
        return a.reshape(T, 8 * n_stripes, n_groups * Dh)

    prologue, point = _schedule(T, n_stripes, B * Sq, D // 8, H * Dh // 128)
    steady = [point(0, 0), point(0, 1)]
    n_steady = 0
    while all(point(n_steady, hf) == [((c[0], c[1] + n_steady) + c[2:], q) for c, q in steady[hf]]
              for hf in (0, 1)):
        n_steady += 1

    K_SEM, V_SEM = 0, _NBUF
    X_SEM, WQ_SEM, WO_SEM, OUT_SEM, LAST_SEM = range(2 * _NBUF, 2 * _NBUF + 5)

    def kernel(x_hbm, k_hbm, v_hbm, wq_hbm, wo_hbm, out_hbm,
               k_buf, v_buf, x_buf, wq_buf, wo_buf, acc, out_buf, q_buf, o_buf, sem):

        def start(c, queue, shift=0):
            if c[0] == 'x':
                src, dst, s = x_hbm.at[pl.ds(c[1], c[2])], x_buf.at[pl.ds(c[1], c[2])], X_SEM
            else:
                rows, cols = pl.ds(8 * c[-3], 8), pl.ds(128 * c[-2], 128 * c[-1])
                if c[0] in 'kv':
                    hbm, buf, s0 = (k_hbm, k_buf, K_SEM) if c[0] == 'k' else (v_hbm, v_buf, V_SEM)
                    hd = c[1] + shift
                    slot = hd & (_NBUF - 1)
                    src, dst, s = hbm.at[hd, rows, cols], buf.at[slot, rows, cols], s0 + slot
                else:
                    hbm, buf, s = (wq_hbm, wq_buf, WQ_SEM) if c[0] == 'wq' else (wo_hbm, wo_buf, WO_SEM)
                    src, dst = hbm.at[rows, cols], buf.at[rows, cols]
            pltpu.make_async_copy(src, dst, sem.at[s]).start(priority=queue)

        def wait_full(buf, s):
            pltpu.make_async_copy(buf, buf, sem.at[s]).wait()

        def write_back(lo, n, s):
            return pltpu.make_async_copy(out_buf.at[pl.ds(lo, n)], out_hbm.at[pl.ds(lo, n)], sem.at[s])

        def issue(t, half):
            def tail(lo, hi):
                if hi - lo == 1:
                    for c, queue in point(lo, half):
                        start(c, queue)
                    return
                mid = (lo + hi) // 2
                if any(point(u, half) for u in range(lo, mid)):
                    pl.when(t < mid)(lambda: tail(lo, mid))
                if any(point(u, half) for u in range(mid, hi)):
                    pl.when(t >= mid)(lambda: tail(mid, hi))

            @pl.when(t < n_steady)
            def _():
                for c, queue in steady[half]:
                    start(c, queue, t)

            pl.when(t >= n_steady)(lambda: tail(n_steady, T))

        def slices(t):
            if isinstance(t, int):
                return pl.ds(t // H * Sq, Sq), pl.ds(t % H * Dh, Dh)
            b, h = jax.lax.shift_right_logical(t, H.bit_length() - 1), t & (H - 1)
            return pl.ds(pl.multiple_of(b * Sq, 16), Sq), pl.ds(pl.multiple_of(h * Dh, Dh), Dh)

        def keys(buf, slot):
            return jnp.concatenate([buf[slot, :, g * Dh:(g + 1) * Dh] for g in range(n_groups)], axis=0)

        def project_q(t):
            rows, cols = slices(t)
            q = jnp.dot(x_buf[rows, :], wq_buf[:, cols], preferred_element_type=jnp.float32)
            q_buf[...] = (q * q_scale).astype(q_buf.dtype)

        def project_out(t, first_head):
            rows, cols = slices(t)
            y = jax.lax.dot_general(o_buf[...], wo_buf[:, cols], (((1,), (1,)), ((), ())),
                                    preferred_element_type=jnp.float32)
            total = y + jnp.where(first_head, 0.0, acc[...])
            if not isinstance(t, int):
                acc[...] = total
            out_buf[rows, :] = total.astype(out_buf.dtype)

        for c, queue in prologue:
            start(c, queue)
        acc[...] = jnp.zeros(acc.shape, acc.dtype)
        o_buf[...] = jnp.zeros(o_buf.shape, o_buf.dtype)
        wait_full(x_buf, X_SEM)
        wait_full(wq_buf, WQ_SEM)
        project_q(0)
        wait_full(wo_buf, WO_SEM)

        def step(t, carry):
            slot = t & (_NBUF - 1)
            prev = jnp.maximum(t - 1, 0)

            wait_full(k_buf.at[slot], K_SEM + slot)
            issue(t, 0)
            s = jax.lax.dot_general(q_buf[...], keys(k_buf, slot), (((1,), (1,)), ((), ())),
                                    preferred_element_type=jnp.float32)
            m = jnp.max(s, axis=-1, keepdims=True)
            project_q(jnp.minimum(t + 1, T - 1))
            project_out(prev, (prev & (H - 1)) == 0)

            @pl.when(t == T - 1)
            def _():
                write_back(0, n_early, OUT_SEM).start(priority=1)

            wait_full(v_buf.at[slot], V_SEM + slot)
            issue(t, 1)
            p = jnp.exp(s - m)
            l = jnp.sum(p, axis=-1, keepdims=True)
            o = jnp.dot(p.astype(v_buf.dtype), keys(v_buf, slot), preferred_element_type=jnp.float32)
            o_buf[...] = (o / l).astype(o_buf.dtype)
            return carry

        jax.lax.fori_loop(0, T, step, 0)
        project_out(T - 1, H == 1)
        write_back(n_early, Sq, LAST_SEM).start()
        write_back(0, n_early, OUT_SEM).wait()
        write_back(n_early, Sq, LAST_SEM).wait()

    hbm = pl.BlockSpec(memory_space=pltpu.MemorySpace.HBM)
    kv_buf = pltpu.VMEM((_NBUF, 8 * n_stripes, n_groups * Dh), k_cache.dtype)
    out = pl.pallas_call(
        kernel,
        in_specs=[hbm] * 5,
        out_specs=hbm,
        out_shape=jax.ShapeDtypeStruct((B * Sq, D), x.dtype),
        scratch_shapes=[
            kv_buf,
            kv_buf,
            pltpu.VMEM((B * Sq, D), x.dtype),
            pltpu.VMEM((D, H * Dh), wq.dtype),
            pltpu.VMEM((D, H * Dh), wo.dtype),
            pltpu.VMEM((Sq, D), jnp.float32),
            pltpu.VMEM((B * Sq, D), x.dtype),
            pltpu.VMEM((Sq, Dh), k_cache.dtype),
            pltpu.VMEM((Sq, Dh), wo.dtype),
            pltpu.SemaphoreType.DMA((LAST_SEM + 1,)),
        ],
        compiler_params=pltpu.CompilerParams(
            vmem_limit_bytes=100 * 1024 * 1024,
            disable_bounds_checks=True,
            disable_semaphore_checks=True,
        ),
    )(x.reshape(B * Sq, D), wide(k_cache), wide(v_cache), wq, wo.T)
    return out.reshape(B, Sq, D)
```

```python
import jax
import jax.numpy as jnp
import jax.experimental.pallas as pl
import jax.experimental.pallas.tpu as pltpu

_STRIPE = 32
_PHASE = 13
_NBUF = 8
_LEAD = 26
_AHEAD = 56
_X_ROWS = 48
_X_Q0 = 4
_W_STREAMS = 4
_DEPTHS = ((7, 1), (18, 2), (1 << 30, 4))
_N_SERIAL = 2
_COST_A, _COST_B = 16, 13


def _kv_order(n_heads, n_stripes):
    def visit(hd, s):
        nxt = (hd, s + 1) if s + 1 < n_stripes else (hd + 1, 0)
        both = [(hd, s, _PHASE, _STRIPE - _PHASE), nxt + (0, _PHASE)]
        return [p for p in both if 0 <= p[0] < n_heads]

    def depth(hd):
        return next(d for n, d in _DEPTHS if n_heads - hd <= n)

    half, deepest = n_stripes // 2, _DEPTHS[-1][1]
    order = visit(-1, n_stripes - 1)
    for g in range(1 - deepest, n_heads):
        work = []
        for i in range(2):
            for w in range(deepest):
                hd = g + w
                if 0 <= hd < n_heads and w < depth(hd):
                    lo, hi = w * half // depth(hd), (w + 1) * half // depth(hd)
                    for j in range(lo, hi):
                        work.append(((j - lo + 0.5) / (hi - lo), len(work), visit(hd, i * half + j)))
        order += [p for _, _, v in sorted(work) for p in v]
    return order


def _schedule(n_heads, n_stripes, x_rows, w_rows):
    xs = [('x', r, min(_X_ROWS, x_rows - r)) for r in range(0, x_rows, _X_ROWS)]

    def w_visit(i):
        both = [(i, _PHASE, _STRIPE - _PHASE), (i + 1, 0, _PHASE)]
        return [p for p in both if 0 <= p[0] < w_rows]

    band = w_rows // _W_STREAMS
    ws = w_visit(-1) + [p for j in range(band) for i in range(_W_STREAMS) for p in w_visit(i * band + j)]
    order = _kv_order(n_heads, n_stripes)
    serial = n_heads - _N_SERIAL
    q0 = [None] * _LEAD + xs[:_X_Q0] + [('wq',) + p for p in ws] + [('k',) + p for p in order if p[0] < serial]
    q1 = xs[_X_Q0:] + [('wo',) + p for p in ws] + [('v',) + p for p in order if p[0] < serial]
    cut = len(q0) - _LEAD
    rest, q1 = q1[cut:], q1[:cut]
    for hd in range(serial, n_heads):
        rest += [(a,) + p for a in 'kv' for p in order if p[0] == hd]
    rest.sort(key=lambda c: c[:2] == ('v', n_heads - 1) and c[3] == 0)
    shared, alone = rest[:-_LEAD], rest[-_LEAD:]
    q0 += [c for c in shared if c[2] < n_stripes // 2]
    q1 += [c for c in shared if c[2] >= n_stripes // 2] + alone
    n_slots = max(len(q0), len(q1))
    slots = [[(q[f], i) for i, q in enumerate((q0, q1)) if f < len(q) and q[f]] for f in range(n_slots)]

    ready = {}
    for f, s in enumerate(slots):
        for c, queue in s:
            ready[c[:2]] = max(ready.get(c[:2], 0), f + 1 - (_LEAD if queue == 0 else 0))
    upto, now = [], 0
    for t in range(n_heads):
        now = max(now, ready['k', t])
        upto.append(now + _AHEAD)
        now = max(now + _COST_A, ready['v', t])
        upto.append(now + _AHEAD)
        now += _COST_B
    upto[0] = upto[2] - 2 * n_stripes
    first = upto[1] - 2 * n_stripes
    upto = [first] + [min(u, n_slots) for u in upto[:-2]] + [n_slots, n_slots]

    def point(t, half):
        return [c for s in slots[upto[2 * t + half]:upto[2 * t + half + 1]] for c in s]

    prologue = [c for s in slots[:first] for c in s]
    assert upto == sorted(upto) and band * _W_STREAMS == w_rows
    assert all(c[1] < _NBUF for c, _ in prologue if c[0] in ('k', 'v'))
    for t in range(n_heads):
        for half in (0, 1):
            for c, _ in point(t, half):
                assert c[0] in ('k', 'v') and c[1] - _NBUF < t
                assert c[1] > t or (c[0] == 'v' and c[1] == t and half == 0)
    for a in ('k', 'v'):
        at = 0
        for hd, row, lo, n in sorted(c[1:] for s in slots for c, _ in s if c[0] == a):
            assert (hd * n_stripes + row) * _STRIPE + lo == at
            at += n
        assert at == n_heads * n_stripes * _STRIPE
    return prologue, point


@jax.jit
def pallas_standalone__mha_block_cached__near_ridge_kernel(
    x: jax.Array,
    k_cache: jax.Array,
    v_cache: jax.Array,
    wq: jax.Array,
    wo: jax.Array,
):
    B, Sq, D = x.shape
    _, H, Sk, Dh = k_cache.shape
    T = B * H
    width = _STRIPE * 128
    n_groups = width // Dh
    n_stripes = Sk // (8 * n_groups)
    n_early = (B - 1) * Sq
    assert H > 2 and H & (H - 1) == 0 and H * Dh == width and Sq % 16 == 0 and D % 8 == 0

    def wide(a):
        a = a.reshape(T, n_stripes, n_groups, 8, Dh).transpose(0, 1, 3, 2, 4)
        return a.reshape(T, 8 * n_stripes, width)

    prologue, point = _schedule(T, n_stripes, B * Sq, D // 8)
    steady = [point(0, 0), point(0, 1)]
    n_steady = 0
    while all(point(n_steady, hf) == [((c[0], c[1] + n_steady) + c[2:], q) for c, q in steady[hf]]
              for hf in (0, 1)):
        n_steady += 1
    assert n_steady + _NBUF <= T

    K_SEM, V_SEM = 0, _NBUF
    X_SEM, WQ_SEM, WO_SEM, LATE_SEM, OUT_SEM, LAST_SEM = range(2 * _NBUF, 2 * _NBUF + 6)

    def kernel(x_hbm, k_hbm, v_hbm, wq_hbm, wo_hbm, out_hbm,
               k_buf, v_buf, x_buf, wq_buf, wo_buf, acc, out_buf, q_buf, o_buf, o_part, sem):

        def start(c, queue, shift=0):
            if c[0] == 'x':
                src, dst, s = x_hbm.at[pl.ds(c[1], c[2])], x_buf.at[pl.ds(c[1], c[2])], X_SEM
            else:
                rows, cols = pl.ds(8 * c[-3], 8), pl.ds(128 * c[-2], 128 * c[-1])
                if c[0] in ('k', 'v'):
                    hbm, buf, s0 = (k_hbm, k_buf, K_SEM) if c[0] == 'k' else (v_hbm, v_buf, V_SEM)
                    hd = c[1] + shift
                    slot = hd & (_NBUF - 1)
                    src, dst, s = hbm.at[hd, rows, cols], buf.at[slot, rows, cols], s0 + slot
                    if c[:2] == ('v', T - 1) and c[-2] == 0:
                        s = LATE_SEM
                else:
                    hbm, buf, s = (wq_hbm, wq_buf, WQ_SEM) if c[0] == 'wq' else (wo_hbm, wo_buf, WO_SEM)
                    src, dst = hbm.at[rows, cols], buf.at[rows, cols]
            pltpu.make_async_copy(src, dst, sem.at[s]).start(priority=queue)

        def wait_full(buf, s):
            pltpu.make_async_copy(buf, buf, sem.at[s]).wait()

        def write_back(lo, n, s):
            return pltpu.make_async_copy(out_buf.at[pl.ds(lo, n)], out_hbm.at[pl.ds(lo, n)], sem.at[s])

        def issue(t, half):
            def tail(lo, hi):
                if hi - lo == 1:
                    for c, queue in point(lo, half):
                        start(c, queue)
                    return
                mid = (lo + hi) // 2
                if any(point(u, half) for u in range(lo, mid)):
                    pl.when(t < mid)(lambda: tail(lo, mid))
                if any(point(u, half) for u in range(mid, hi)):
                    pl.when(t >= mid)(lambda: tail(mid, hi))

            @pl.when(t < n_steady)
            def _():
                for c, queue in steady[half]:
                    start(c, queue, t)

            pl.when(t >= n_steady)(lambda: tail(n_steady, T - 1))

        def slices(t):
            if isinstance(t, int):
                return pl.ds(t // H * Sq, Sq), pl.ds(t % H * Dh, Dh)
            b, h = jax.lax.shift_right_logical(t, H.bit_length() - 1), t & (H - 1)
            return pl.ds(pl.multiple_of(b * Sq, 16), Sq), pl.ds(pl.multiple_of(h * Dh, Dh), Dh)

        def keys(a):
            return jnp.concatenate([a[:, g:g + Dh] for g in range(0, a.shape[1], Dh)], axis=0)

        def scores(slot):
            s = jax.lax.dot_general(q_buf[...], keys(k_buf[slot]), (((1,), (1,)), ((), ())),
                                    preferred_element_type=jnp.float32)
            return s, jnp.max(s, axis=-1, keepdims=True)

        def weights(s, m):
            p = jnp.exp(s - m)
            return p.astype(v_buf.dtype), jnp.sum(p, axis=-1, keepdims=True)

        def project_q(t):
            rows, cols = slices(t)
            q = jnp.dot(x_buf[rows, :], wq_buf[:, cols], preferred_element_type=jnp.float32)
            q_buf[...] = (q * Dh ** -0.5).astype(q_buf.dtype)

        def project_out(t, first_head, keep=True):
            rows, cols = slices(t)
            y = jax.lax.dot_general(o_buf[...], wo_buf[:, cols], (((1,), (1,)), ((), ())),
                                    preferred_element_type=jnp.float32)
            total = y + jnp.where(first_head, 0.0, acc[...])
            if keep:
                acc[...] = total
            out_buf[rows, :] = total.astype(out_buf.dtype)

        for c, queue in prologue:
            start(c, queue)
        acc[...] = jnp.zeros(acc.shape, acc.dtype)
        o_buf[...] = jnp.zeros(o_buf.shape, o_buf.dtype)
        wait_full(x_buf, X_SEM)
        wait_full(wq_buf, WQ_SEM)
        project_q(0)
        wait_full(wo_buf, WO_SEM)

        def step(t, carry):
            slot = t & (_NBUF - 1)
            prev = jnp.maximum(t - 1, 0)

            wait_full(k_buf.at[slot], K_SEM + slot)
            issue(t, 0)
            s, m = scores(slot)
            project_q(t + 1)
            project_out(prev, (prev & (H - 1)) == 0)

            wait_full(v_buf.at[slot], V_SEM + slot)
            issue(t, 1)
            p, l = weights(s, m)
            o = jnp.dot(p, keys(v_buf[slot]), preferred_element_type=jnp.float32)
            o_buf[...] = (o / l).astype(o_buf.dtype)
            return carry

        jax.lax.fori_loop(0, T - 1, step, 0)

        slot = (T - 1) % _NBUF
        cut = _PHASE * 128
        late_cols = -(-cut // Dh) * Dh
        late_keys = late_cols // Dh * 8 * n_stripes
        wait_full(k_buf.at[slot], K_SEM + slot)
        for c, queue in point(T - 1, 0):
            start(c, queue)
        s, m = scores(slot)
        project_out(T - 2, False)
        write_back(0, n_early, OUT_SEM).start(priority=1)
        wait_full(v_buf.at[slot, :, pl.ds(cut, width - cut)], V_SEM + slot)
        p, l = weights(s, m)
        o_part[...] = jnp.dot(p[:, late_keys:], keys(v_buf[slot, :, late_cols:]),
                              preferred_element_type=jnp.float32)
        wait_full(v_buf.at[slot, :, pl.ds(0, cut)], LATE_SEM)
        o = o_part[...] + jnp.dot(p[:, :late_keys], keys(v_buf[slot, :, :late_cols]),
                                  preferred_element_type=jnp.float32)
        o_buf[...] = (o / l).astype(o_buf.dtype)
        project_out(T - 1, False, keep=False)
        write_back(n_early, Sq, LAST_SEM).start()
        write_back(0, n_early, OUT_SEM).wait()
        write_back(n_early, Sq, LAST_SEM).wait()

    hbm = pl.BlockSpec(memory_space=pltpu.MemorySpace.HBM)
    kv_buf = pltpu.VMEM((_NBUF, 8 * n_stripes, width), k_cache.dtype)
    out = pl.pallas_call(
        kernel,
        in_specs=[hbm] * 5,
        out_specs=hbm,
        out_shape=jax.ShapeDtypeStruct((B * Sq, D), x.dtype),
        scratch_shapes=[
            kv_buf,
            kv_buf,
            pltpu.VMEM((B * Sq, D), x.dtype),
            pltpu.VMEM((D, width), wq.dtype),
            pltpu.VMEM((D, width), wo.dtype),
            pltpu.VMEM((Sq, D), jnp.float32),
            pltpu.VMEM((B * Sq, D), x.dtype),
            pltpu.VMEM((Sq, Dh), k_cache.dtype),
            pltpu.VMEM((Sq, Dh), wo.dtype),
            pltpu.VMEM((Sq, Dh), jnp.float32),
            pltpu.SemaphoreType.DMA((LAST_SEM + 1,)),
        ],
        compiler_params=pltpu.CompilerParams(
            vmem_limit_bytes=100 * 1024 * 1024,
            disable_bounds_checks=True,
            disable_semaphore_checks=True,
        ),
    )(x.reshape(B * Sq, D), wide(k_cache), wide(v_cache), wq, wo.T)
    return out.reshape(B, Sq, D)
```
